```python
import os as _os
_os.environ.setdefault("JAX_PLATFORMS", "cpu")
import jax
import jax.numpy as jnp

def _softmax(x, axis=-1):
    return jax.nn.softmax(x, axis=axis)
def _gelu(x):
    return jax.nn.gelu(x, approximate=True)
def _silu(x):
    return jax.nn.silu(x)
def _sigmoid(x):
    return jax.nn.sigmoid(x)
def _layernorm(x, axis=-1, eps=1e-5):
    m = jnp.mean(x, axis=axis, keepdims=True)
    v = jnp.var(x, axis=axis, keepdims=True)
    return (x - m) / jnp.sqrt(v + eps)
def _scatter_add(tgt, idx, src, axis=0):
    return tgt.at[idx].add(src)
def _segment_sum(src, seg, n):
    return jax.ops.segment_sum(src, seg, n)
class _Rng:
    def __init__(self, key):
        self._k = key
    def _next(self):
        self._k, sub = jax.random.split(self._k)
        return sub
    def normal(self, shape):
        return jax.random.normal(self._next(), shape, dtype=jnp.bfloat16)
    def randint(self, lo, hi, shape):
        return jax.random.randint(self._next(), shape, lo, hi, dtype=jnp.int32)
    def uniform(self, shape, lo=0.0, hi=1.0):
        return jax.random.uniform(self._next(), shape, jnp.bfloat16, lo, hi)
    def permutation(self, n):
        return jax.random.permutation(self._next(), n)


kernel_name = 'recurrent_scan__ssm_conv_s4__mixer_s_mlp__prompt'

def setup_inputs():
    _rng = _Rng(jax.random.key(int.from_bytes(__import__("os").urandom(4), "little")))
    _w = (lambda a: (lambda t: t.astype(jnp.bfloat16) if jnp.issubdtype(t.dtype, jnp.floating) else t)(jnp.asarray(a)))
    def _A_setup():
        B, L, D, N = 1, 2048, 512, 128
        A_re = -jnp.exp((lambda *s: _rng.normal(s) * 0.1)(D, N))
        A_im = jnp.pi * (lambda *s: _rng.normal(s) * 0.1)(D, N)
        B_re = (lambda *s: _rng.normal(s) * 0.1)(D, N)
        B_im = (lambda *s: _rng.normal(s) * 0.1)(D, N)
        C_re = (lambda *s: _rng.normal(s) * 0.1)(D, N)
        C_im = (lambda *s: _rng.normal(s) * 0.1)(D, N)
        log_dt = (lambda *s: _rng.normal(s) * 0.1)(D) * 0.5 - 4.0
        Dskip = (lambda *s: _rng.normal(s) * 0.05)(D)
        return {
            "u": _w((lambda *s: _rng.normal(s) * 0.05)(B, L, D)),
            "A_re": _w(A_re),
            "A_im": _w(A_im),
            "B_re": _w(B_re),
            "B_im": _w(B_im),
            "C_re": _w(C_re),
            "C_im": _w(C_im),
            "log_dt": _w(log_dt),
            "Dskip": _w(Dskip),
        }
    _A_in = _A_setup()

    def _B_setup():
        B, S, D, F = 1, 2048, 512, 1376
        return {
            "x":  _w((lambda *s: _rng.normal(s) * 0.05)(B, S, D)),
            "w1": _w((lambda *s: _rng.normal(s) * 0.8)(D, D) * (D ** -0.5)),
            "w2": _w((lambda *s: _rng.normal(s) * 0.8)(D, D) * (D ** -0.5)),
            "w3": _w((lambda *s: _rng.normal(s) * 0.8)(D, F) * (D ** -0.5)),
            "w4": _w((lambda *s: _rng.normal(s) * 0.8)(F, D) * (F ** -0.5)),
        }
    _B_in = _B_setup()

    return {
        "A_u": _A_in["u"],
        "A_A_re": _A_in["A_re"],
        "A_A_im": _A_in["A_im"],
        "A_B_re": _A_in["B_re"],
        "A_B_im": _A_in["B_im"],
        "A_C_re": _A_in["C_re"],
        "A_C_im": _A_in["C_im"],
        "A_log_dt": _A_in["log_dt"],
        "A_Dskip": _A_in["Dskip"],
        "B_x": _B_in["x"],
        "B_w1": _B_in["w1"],
        "B_w2": _B_in["w2"],
        "B_w3": _B_in["w3"],
        "B_w4": _B_in["w4"],
    }

def reference(A_u, A_A_re, A_A_im, A_B_re, A_B_im, A_C_re, A_C_im, A_log_dt, A_Dskip, B_x, B_w1, B_w2, B_w3, B_w4):
    def _A_ref(u, A_re, A_im, B_re, B_im, C_re, C_im, log_dt, Dskip):
        Bsz, L, D = u.shape
        dt = jnp.exp(log_dt)[:, None]
        A = A_re + 1j * A_im
        Bc = B_re + 1j * B_im
        Cc = C_re + 1j * C_im
        logdA = dt * A
        dB = dt * Bc
        l = (lambda x, dt: x.astype(dt))(jnp.arange(L), A_re.dtype)
        P = jnp.exp(logdA[:, :, None] * l[None, None, :])
        K = jnp.einsum("dn,dnl,dn->dl", Cc, P, dB).real
        L2 = 2 * L
        Kp = jnp.pad(K, ((0, 0), (0, L)))
        up = (lambda x, *d: x.transpose(*d))(u, 0, 2, 1)
        up = jnp.pad(up, ((0, 0), (0, 0), (0, L)))
        Kf = (lambda x, axes=(-2,-1): jnp.fft.rfft2(x.astype(jnp.float32), axes=axes))(Kp[:, None, :], axes=(-2, -1))
        Uf = (lambda x, axes=(-2,-1): jnp.fft.rfft2(x.astype(jnp.float32), axes=axes))(up[:, :, None, :], axes=(-2, -1))
        Yf = Uf * Kf[None, :, :, :]
        y = (lambda x, s, axes=(-2,-1): jnp.fft.irfft2(x, s=s, axes=axes).astype(jnp.bfloat16))(Yf, (1, L2), axes=(-2, -1))[:, :, 0, :L]
        y = (lambda x, *d: x.transpose(*d))(y, 0, 2, 1) + u * Dskip[None, None, :]
        return y

    def _B_ref(x, w1, w2, w3, w4):
        B, S, D = x.shape
        h = _gelu(_layernorm(x, axis=-1) @ w1)
        c = D // 4
        g0 = jnp.pad(h[:, :, 0*c:1*c], ((0, 0), (1, 0), (0, 0)))[:, :S, :]
        g1 = jnp.pad(h[:, :, 1*c:2*c], ((0, 0), (0, 1), (0, 0)))[:, 1:, :]
        g2 = jnp.pad(h[:, :, 2*c:3*c], ((0, 0), (2, 0), (0, 0)))[:, :S, :]
        g3 = jnp.pad(h[:, :, 3*c:   ], ((0, 0), (0, 2), (0, 0)))[:, 2:, :]
        hs = jnp.concatenate([g0, g1, g2, g3], axis=-1) @ w2
        x1 = x + hs
        h2 = _gelu(_layernorm(x1, axis=-1) @ w3) @ w4
        return x1 + h2

    x = A_u
    xn = _layernorm(x, axis=-1)
    s = _A_ref(xn, A_A_re, A_A_im, A_B_re, A_B_im, A_C_re, A_C_im, A_log_dt, A_Dskip)
    g = _silu(_B_ref(xn, B_w1, B_w2, B_w3, B_w4))
    return x + s * g
```

```python
import jax
import jax.numpy as jnp
from jax import lax
import jax.experimental.pallas as pl
import jax.experimental.pallas.tpu as pltpu

L, D, N, F = 2048, 512, 128, 1376
TM = 256
NT = L // TM
GPI = 8
FCH = [(i, min(128, F - i)) for i in range(0, F, 128)]
SKEW, PRE, NS, KB = 2, 6, 6, [(i, 256) for i in range(0, 1280, 256)] + [(1280, 96)]
LAG = 3
f32, bf16 = jnp.float32, jnp.bfloat16


def _ln(x):
    m = jnp.mean(x, axis=-1, keepdims=True)
    c = x - m
    v = jnp.mean(c * c, axis=-1, keepdims=True)
    return c * lax.rsqrt(v + 1e-5)


def _gelu(x):
    k = 0.7978845608028654
    t = jnp.tanh(x * (k + (k * 0.044715) * (x * x)))
    hx = 0.5 * x
    return hx + hx * t


def _cmul(a, b):
    return a[0] * b[0] - a[1] * b[1], a[0] * b[1] + a[1] * b[0]


def _column(ref):
    row = ref[...].astype(f32).reshape(1, D)
    return [jnp.broadcast_to(row[:, i * 128:(i + 1) * 128], (128, 128)).T for i in range(4)]


def _ssm_group(g, prm, dt_ref, ut, yt, pw, st, tb, cs, tab_all, gen):
    cs = cs.at[:, pl.ds(pl.multiple_of(g * 8, 8), 8), :]
    if gen:
        tb = tb
    are, aim, bre, bim, cre, cim = prm
    def prelim():
        r8 = pl.ds(pl.multiple_of(g * 8, 8), 8)
        dt = dt_ref[r8, :]
        mag = jnp.exp(dt * are[r8, :].astype(f32))
        th = dt * aim[r8, :].astype(f32)
        lam = (mag * jnp.cos(th), mag * jnp.sin(th))
        B = (bre[r8, :].astype(f32), bim[r8, :].astype(f32))
        C = (cre[r8, :].astype(f32), cim[r8, :].astype(f32))
        cb = _cmul(C, B)
        cb = (cb[0] * dt, cb[1] * dt)
        w = _cmul(cb, lam)
        p = None
        for b in range(17):
            p = (jnp.ones_like(dt), jnp.zeros_like(dt)) if b == 0 else (lam if b == 1 else _cmul(p, lam))
            slot = b if b == 16 else (b % 2) * 8 + b // 2
            pw[0, pl.ds(slot, 8, stride=17), :] = p[0]
            pw[1, pl.ds(slot, 8, stride=17), :] = p[1]
        big = p
        for _ in range(3):
            big = (big[0] * big[0] - big[1] * big[1], 2.0 * big[0] * big[1])
        for n, x in enumerate(cb + w + big):
            cs[n] = x
    if gen:
        prelim()
    yield
    base = pl.multiple_of(g * 72, 8)
    for ch in range(8 if gen else 0):
        v = [tuple(pw[q, pl.ds(17 * ch + 8 * h, 8), :] for q in range(2)) for h in range(2)]
        m = tuple(jnp.broadcast_to(pw[q, pl.ds(17 * ch + 16, 1), :], (8, 128)) for q in range(2))
        for a in range(8):
            for q in range(2):
                tb[ch, 8 * a:8 * a + 8, 128 * q:128 * q + 128] = pltpu.pack_elementwise(
                    [v[0][q], v[1][q]], packed_dtype=bf16)
            v = [_cmul(x, m) for x in v]
        tab = pltpu.bitcast(tb[ch], bf16)
        u = pltpu.bitcast(ut[pl.ds(base + 9 * ch, 8), :], bf16)
        s = jnp.dot(u, tab, preferred_element_type=f32)
        st[0, pl.ds(ch, 16, stride=9), :] = s[:, :128]
        st[1, pl.ds(ch, 16, stride=9), :] = s[:, 128:]
        yield
    cb, w, big = (cs[0], cs[1]), (cs[2], cs[3]), (cs[4], cs[5])
    yield
    h = cb
    for c in range(16):
        st[2, pl.ds(9 * c, 8), :] = h[0]
        st[3, pl.ds(9 * c, 8), :] = -h[1]
        if c < 15:
            s = _cmul(w, (st[0, pl.ds(9 * c, 8), :], st[1, pl.ds(9 * c, 8), :]))
            if c > 0:
                t = _cmul(big, h)
                s = (s[0] + t[0], s[1] + t[1])
            h = s
        if c % 8 == 7:
            yield
    row16 = lax.broadcasted_iota(jnp.int32, (16, 128), 0)
    lane16 = lax.broadcasted_iota(jnp.int32, (16, 128), 1)
    rev = 7 - lax.broadcasted_iota(jnp.int32, (8, 128), 0)
    yield
    R = range(8)
    ys = []
    for ch in R:
        ys.append(lax.dot_general(
            jnp.concatenate([st[2, pl.ds(ch, 16, stride=9), :], st[3, pl.ds(ch, 16, stride=9), :]], 1).astype(bf16),
            pltpu.bitcast(tb[ch], bf16), (((1,), (1,)), ((), ())), preferred_element_type=f32))
        if ch % 2:
            yield
    k16 = []
    for y in ys:
        k = pltpu.roll(jnp.broadcast_to(y[0:1, :], (8, 128)), 0, 1, stride=2, stride_axis=0)
        k16.append(jnp.take_along_axis(k, rev, axis=0))
    yield
    k16 = [pltpu.bitcast(pltpu.pack_elementwise([pltpu.roll(k, 1, 1), k], packed_dtype=bf16), jnp.int32) for k in k16]
    yield
    roll7 = lambda ch: [pltpu.roll(k16[ch], 112 - 16 * a, 1) for a in range(7)] + [k16[ch]]
    rl = [roll7(0), roll7(1)]

    def intra(ch):
        u = pltpu.bitcast(ut[pl.ds(base + 9 * ch, 8), :], bf16)
        ys[ch] = jnp.where(row16 == 0, 0.0, ys[ch]) + jnp.dot(u, pltpu.bitcast(tb[ch, :, 0:128], bf16), preferred_element_type=f32)

    q8 = (lax.broadcasted_iota(jnp.int32, (8, 128), 1) + 2 * lax.broadcasted_iota(jnp.int32, (8, 128), 0))
    for ch in R:
        if ch < 6:
            rl.append(roll7(ch + 2))
        for a in range(8):
            t = q8 - (126 - 16 * a)
            keep = jnp.where(t >= 1, -1, jnp.where(t >= 0, -65536, 0))
            r = rl[ch][a]
            tb[ch, 8 * a:8 * a + 8, 0:128] = pltpu.bitcast(r & keep, jnp.uint32)
        if ch >= 2:
            intra(ch - 2)
        if ch > LAG + 1:
            yt[pl.ds(base + 9 * (ch - 2 - LAG), 8), :] = pltpu.bitcast(ys[ch - 2 - LAG].astype(bf16), jnp.uint32)
        yield
    intra(6)
    intra(7)
    yield
    for ch in range(6 - LAG, 8):
        yt[pl.ds(base + 9 * ch, 8), :] = pltpu.bitcast(ys[ch].astype(bf16), jnp.uint32)


def _kernel(u_hbm, are, aim, bre, bim, cre, cim, ldt_ref, dsk_ref, w1h, w2h, w3h, w4h, o_hbm,
            u, w1, w2, w3t, w4, w3, xn_s, xa_s, h0, h1, h2, h3, ut, yt, e_s, g_s, dt_s, ob, sem_u, sem_w, sem_o, cs, tab_all, *pws):
    hs = (h0, h1, h2, h3)

    def u_cp(i):
        r = pl.ds(i * TM, TM)
        return pltpu.make_async_copy(u_hbm.at[0, r], u.at[r], sem_u.at[i])

    def o_cp(i):
        r = pl.ds(i * TM, TM)
        return pltpu.make_async_copy(ob.at[r], o_hbm.at[0, r], sem_o.at[i])

    wcp = [pltpu.make_async_copy(a, b, sem_w.at[i])
           for i, (a, b) in enumerate(((w1h, w1), (w2h, w2), (w3h, w3t), (w4h, w4)))]
    u_cp(0).start()
    wcp[0].start()
    wcp[1].start()
    for i in range(1, NT):
        u_cp(i).start()
    for c in wcp[2:]:
        c.start()
    for i, c in enumerate(_column(ldt_ref)):
        dt_s[i * 128:(i + 1) * 128, :] = jnp.exp(c).astype(bf16).astype(f32)
    for h in hs:
        h[0:8, :] = jnp.zeros((8, 128), f32)
        h[TM + 8:TM + 16, :] = jnp.zeros((8, 128), f32)
        h[L + 8:L + 16, :] = jnp.zeros((8, 128), f32)
    wcp[0].wait()
    wcp[1].wait()

    def mix(i):
        r0 = pl.multiple_of(i * TM, TM)
        hin = jnp.concatenate([hs[b][pl.ds(r0 + 8 + s, TM), :] for b, s in enumerate((-1, 1, -2, 2))], 1)
        x1 = xn_s[pl.ds(r0, TM), :].astype(f32) + jnp.dot(hin.astype(bf16), w2[...], preferred_element_type=f32)
        e_s[pl.ds(r0, TM), :] = x1
        xa_s[pl.ds(r0, TM), :] = _ln(x1).astype(bf16)

    def p1(i, _):
        u_cp(i).wait()
        r0 = pl.multiple_of(i * TM, TM)
        xn = _ln(u[pl.ds(r0, TM), :].astype(f32))
        xb = xn.astype(bf16)
        xn_s[pl.ds(r0, TM), :] = xb
        rev = (7 - lax.broadcasted_iota(jnp.int32, (8, 128), 0))
        r8 = lax.broadcasted_iota(jnp.int32, (8, 128), 0)
        rev = 7 - r8
        xr = xb.astype(f32)
        pk = pltpu.pack_elementwise([xr[:128], xr[128:]], packed_dtype=bf16)
        for b in range(4):
            t = []
            for k in range(112, -16, -16):
                lo, hi = (jnp.take_along_axis(pk[k + o:k + o + 8, b * 128:(b + 1) * 128], rev, axis=0) for o in (8, 0))
                t += [lo, hi]
            t = jnp.concatenate(t, 0)
            ut[pl.ds(b * 128 * 9 + i, 128, stride=9), :] = t.T
        h = _gelu(jnp.dot(_ln(xr).astype(bf16), w1[...], preferred_element_type=f32))
        for b in range(4):
            hs[b][pl.ds(r0 + 8, TM), :] = h[:, b * 128:(b + 1) * 128]
        mix(jnp.maximum(i - 1, 0))
        return 0

    lax.fori_loop(0, NT, p1, 0)
    mix(NT - 1)
    for c in wcp[2:]:
        c.wait()
    for f0, fw in FCH:
        w3[:, f0:f0 + fw] = w3t[f0:f0 + fw, :].T

    def p2(i, _):
        r0 = pl.multiple_of(i * TM, TM)
        acc = e_s[pl.ds(r0, TM), :]
        a = xa_s[pl.ds(r0, TM), :]
        xn = xn_s[pl.ds(r0, TM), :].astype(f32)
        k0 = 0
        for f0, fw in KB:
            t = jnp.dot(a, w3[:, f0:f0 + fw], preferred_element_type=f32)
            pass
            if k0:
                acc = acc + jnp.dot(p, w4[k0 - pw_:k0, :], preferred_element_type=f32)
            p, pw_, k0 = _gelu(t).astype(bf16), fw, f0 + fw
            pass
        acc = acc + jnp.dot(p, w4[k0 - pw_:k0, :], preferred_element_type=f32)
        pass
        g = acc * jax.nn.sigmoid(acc)
        g_s[pl.ds(r0, TM), :] = g
        e_s[pl.ds(r0, TM), :] = u[pl.ds(r0, TM), :].astype(f32) + xn * dsk_ref[...].astype(f32).reshape(1, D) * g
        return 0

    lax.fori_loop(0, NT, p2, 0)

    def p2s(i, _):
        gens = [_ssm_group(i * GPI + q, (are, aim, bre, bim, cre, cim), dt_s, ut, yt, *pws[3 * q:3 * q + 3], cs, None, True)
                for q in range(GPI)]

        clock = [0]

        def step():
            t = clock[0]
            clock[0] += 1
            for q in range(GPI):
                if 0 <= t - q * SKEW:
                    next(gens[q], None)

        for _ in range(40 + GPI * SKEW):
            step()
        return 0

    lax.fori_loop(0, NT, p2s, 0)

    def p3(i, _):
        r0 = pl.multiple_of(i * TM, TM)
        for b in range(4):
            t = yt[pl.ds(b * 128 * 9 + i, 128, stride=9), :].T
            for q in range(2):
                y = pltpu.unpack_elementwise(t, index=q, packed_dtype=bf16, unpacked_dtype=f32)
                rr, cc = pl.ds(r0 + q * 128, 128), slice(b * 128, (b + 1) * 128)
                ob[rr, cc] = (e_s[rr, cc] + y * g_s[rr, cc]).astype(bf16)
        o_cp(i).start()
        return 0

    lax.fori_loop(0, NT, p3, 0)
    for i in range(NT):
        o_cp(i).wait()


@jax.jit
def pallas_recurrent_scan__ssm_conv_s4__mixer_s_mlp__prompt_kernel(
    A_u, A_A_re, A_A_im, A_B_re, A_B_im, A_C_re, A_C_im, A_log_dt, A_Dskip,
    B_x, B_w1, B_w2, B_w3, B_w4,
):
    V = pltpu.VMEM
    hbm = pl.BlockSpec(memory_space=pl.ANY)
    vm = pl.BlockSpec(memory_space=V)
    scratch = [V((L, D), bf16), V((D, D), bf16), V((D, D), bf16), V((F, D), bf16), V((F, D), bf16), V((D, F), bf16),
               V((L, D), bf16), V((L, D), bf16)] + [V((L + 16, 128), f32)] * 4 + [
               V((D * 9, 128), jnp.uint32), V((D * 9, 128), jnp.uint32), V((L, D), f32), V((L, D), f32),
               V((D, 128), f32), V((L, D), bf16),
               pltpu.SemaphoreType.DMA((NT,)), pltpu.SemaphoreType.DMA((4,)), pltpu.SemaphoreType.DMA((NT,))]
    scratch += [V((6, D, 128), f32), V((8, 64, 256), jnp.uint32)]
    scratch += [V((2, 136, 128), f32), V((4, 144, 128), f32), V((8, 64, 256), jnp.uint32)] * GPI
    return pl.pallas_call(
        _kernel,
        in_specs=[hbm] + [vm] * 8 + [hbm] * 4,
        out_specs=hbm,
        out_shape=jax.ShapeDtypeStruct((1, L, D), bf16),
        scratch_shapes=scratch,
        compiler_params=pltpu.CompilerParams(vmem_limit_bytes=100 << 20,
                                             flags={'XLA_TPU_FORCE_LP_LLO_SCHEDULER': True}),
    )(A_u, A_A_re, A_A_im, A_B_re, A_B_im, A_C_re, A_C_im, A_log_dt, A_Dskip, B_w1, B_w2, B_w3.T, B_w4)
```
